```python
import jax
import jax.numpy as jnp

def _softmax(x, axis=-1):
    return jax.nn.softmax(x, axis=axis)
def _gelu(x):
    return jax.nn.gelu(x, approximate=True)
def _silu(x):
    return jax.nn.silu(x)
def _sigmoid(x):
    return jax.nn.sigmoid(x)
def _layernorm(x, axis=-1, eps=1e-5):
    m = jnp.mean(x, axis=axis, keepdims=True)
    v = jnp.var(x, axis=axis, keepdims=True)
    return (x - m) / jnp.sqrt(v + eps)
def _scatter_add(tgt, idx, src, axis=0):
    return tgt.at[idx].add(src)
def _segment_sum(src, seg, n):
    return jax.ops.segment_sum(src, seg, n)
class _Rng:
    def __init__(self, key):
        self._k = key
    def _next(self):
        self._k, sub = jax.random.split(self._k)
        return sub
    def normal(self, shape):
        return jax.random.normal(self._next(), shape, dtype=jnp.bfloat16)
    def randint(self, lo, hi, shape):
        return jax.random.randint(self._next(), shape, lo, hi, dtype=jnp.int32)
    def uniform(self, shape, lo=0.0, hi=1.0):
        return jax.random.uniform(self._next(), shape, jnp.bfloat16, lo, hi)
    def permutation(self, n):
        return jax.random.permutation(self._next(), n)


kernel_name = 'parallel_sum__linear_attn_block__moe_arch_mod__prompt'

def setup_inputs():
    _rng = _Rng(jax.random.key(int.from_bytes(__import__("os").urandom(4), "little")))
    _w = (lambda a: (lambda t: t.astype(jnp.bfloat16) if jnp.issubdtype(t.dtype, jnp.floating) else t)(jnp.asarray(a)))
    def _A_setup():
        B, S, D = 1, 2048, 1024
        return {
            "x": _w((lambda *s: _rng.normal(s) * 0.05)(B, S, D)),
            "wqkv": _w((lambda *s: _rng.normal(s) * 0.05)(D, 3 * D)),
            "wo": _w((lambda *s: _rng.normal(s) * 0.05)(D, D)),
        }
    _A_in = _A_setup()

    def _B_setup():
        B, S, D, F, C = 1, 2048, 1024, 3584, 1
        return {
            "x": _w((lambda *s: _rng.normal(s) * 0.05)(B, S, D)),
            "w_r": _w((lambda *s: _rng.normal(s) * 0.05)(D)),
            "w_gate": _w((lambda *s: _rng.normal(s) * 0.05)(D, F)),
            "w_up": _w((lambda *s: _rng.normal(s) * 0.05)(D, F)),
            "w_down": _w((lambda *s: _rng.normal(s) * 0.05)(F, D)),
        }
    _B_in = _B_setup()

    return {
        "A_x": _A_in["x"],
        "A_wqkv": _A_in["wqkv"],
        "A_wo": _A_in["wo"],
        "B_x": _B_in["x"],
        "B_w_r": _B_in["w_r"],
        "B_w_gate": _B_in["w_gate"],
        "B_w_up": _B_in["w_up"],
        "B_w_down": _B_in["w_down"],
    }

def reference(A_x, A_wqkv, A_wo, B_x, B_w_r, B_w_gate, B_w_up, B_w_down):
    def _A_ref(x, wqkv, wo):
        B, S, D = x.shape
        H = 32; Dh = D // H
        qkv = (lambda x, *d: x.transpose(*d))((x @ wqkv).reshape(B, S, 3, H, Dh), 2, 0, 3, 1, 4)
        q, k, v = qkv[0], qkv[1], qkv[2]
        phi = lambda t: jnp.where(t > 0, t + 1, jnp.exp(t)) + 1e-6
        pq, pk = phi(q), phi(k)
        kv = jnp.einsum("bhsd,bhse->bhde", pk, v)
        z = jnp.einsum("bhsd->bhd", pk)
        num = jnp.einsum("bhqd,bhde->bhqe", pq, kv)
        den = jnp.einsum("bhqd,bhd->bhq", pq, z)[..., None] + 1e-6
        o = num / den
        return (lambda x, *d: x.transpose(*d))(o, 0, 2, 1, 3).reshape(B, S, D) @ wo

    def _B_ref(x, w_r, w_gate, w_up, w_down):
        B, S, D = x.shape
        C = 1
        r = x @ w_r
        idx = jnp.argsort(-r, axis=-1)[:, :C]
        idx_e = jnp.repeat(idx.reshape(B, C, 1), D, axis=2)
        x_sel = jnp.take_along_axis(x, idx_e, axis=1)
        g = _silu(x_sel @ w_gate)
        u = x_sel @ w_up
        y = (g * u) @ w_down
        r_sel = _sigmoid(jnp.take_along_axis(r, idx, axis=1))
        y = y * r_sel.reshape(B, C, 1)
        b_off = (jnp.arange(B) * S).reshape(B, 1)
        flat_idx = (idx + b_off).reshape(B * C)
        zero = (x * 0.0).reshape(B * S, D)
        upd = _scatter_add(zero, flat_idx, y.reshape(B * C, D), axis=0)
        return x + upd.reshape(B, S, D)

    x = A_x
    xn = _layernorm(x, axis=-1)
    return x + _A_ref(xn, A_wqkv, A_wo) + _B_ref(xn, B_w_r, B_w_gate, B_w_up, B_w_down)
```

```python
import contextlib
import numpy as np
import jax
import jax.numpy as jnp
from jax import lax
from jax.experimental import pallas as pl
from jax.experimental.pallas import tpu as pltpu

S, D, NH, DH, F = 2048, 1024, 32, 32, 3584
F32, BF16, I32 = jnp.float32, jnp.bfloat16, jnp.int32


def _dot(a, b):
    return jnp.dot(a, b, preferred_element_type=F32)


def _up(w):
    return pltpu.bitcast(w, BF16)


def _pk2(e, o):
    return pltpu.pack_elementwise([e, o], packed_dtype=BF16)


def _pk_blocks(v):
    m, n = v.shape
    v4 = v.reshape(m // 16, 2, 8, n)
    return _pk2(v4[:, 0], v4[:, 1]).reshape(m // 2, n)


def _unp(w, i):
    return pltpu.unpack_elementwise(w, index=i, packed_dtype=BF16, unpacked_dtype=F32)


def _rcp(d):
    r = pl.reciprocal(d, approx=True)
    return r * (2.0 - d * r)


def _phi(t):
    return jnp.where(t > 0, t + 1.0, jnp.exp(t)) + 1e-6


def _quad(X, i, j):
    h = len(X) // 2
    return [row[j * h:(j + 1) * h] for row in X[i * h:(i + 1) * h]]


def _level(X, aside, add):
    x11, x12, x21, x22 = _quad(X, 0, 0), _quad(X, 0, 1), _quad(X, 1, 0), _quad(X, 1, 1)
    if aside:
        return [add(x11, x22, 1), add(x21, x22, 1), x11, x22, add(x11, x12, 1), add(x21, x11, -1), add(x12, x22, -1)]
    return [add(x11, x22, 1), x11, add(x12, x22, -1), add(x21, x11, -1), x22, add(x11, x12, 1), add(x21, x22, 1)]


def _terms(R, aside):
    sym = [[[(1, a, b)] for b in range(R)] for a in range(R)]
    add = lambda X, Y, sg: [[x + [(sg * s, a, b) for (s, a, b) in y] for x, y in zip(rx, ry)] for rx, ry in zip(X, Y)]

    def rec(X):
        if len(X) == 1:
            return [X[0][0]]
        return [e for o in _level(X, aside, add) for e in rec(o)]
    return rec(sym)


class _Lazy:
    def __init__(self, f):
        self.f, self.v, self.done = f, None, False

    def get(self):
        if not self.done:
            self.v, self.done = self.f(), True
        return self.v


def _lazy_add(X, Y, s):
    if s > 0:
        return [[_Lazy(lambda x=x, y=y: x.get() + y.get()) for x, y in zip(rx, ry)] for rx, ry in zip(X, Y)]
    return [[_Lazy(lambda x=x, y=y: x.get() - y.get()) for x, y in zip(rx, ry)] for rx, ry in zip(X, Y)]


def _operands(blk, aside, out):
    if len(blk) == 1:
        out.append(blk[0][0].get())
        return
    for o in _level(blk, aside, _lazy_add):
        _operands(o, aside, out)


def _strassen(prod, lvl, emit=None, base=0, i0=0, j0=0):
    if lvl == 0:
        v = prod(base)
        if emit is not None:
            emit(i0, j0, v)
            return None
        return [[v]]
    n = 7 ** (lvl - 1)
    h = 2 ** (lvl - 1)
    m = lambda k: _strassen(prod, lvl - 1, None, base + k * n)
    add = lambda X, Y: [[x + y for x, y in zip(rx, ry)] for rx, ry in zip(X, Y)]
    sub = lambda X, Y: [[x - y for x, y in zip(rx, ry)] for rx, ry in zip(X, Y)]
    out = [[None] * (2 * h) for _ in range(2 * h)]

    def fin(qi, qj, X):
        for a in range(h):
            for b in range(h):
                if emit is not None:
                    emit(i0 + qi * h + a, j0 + qj * h + b, X[a][b])
                else:
                    out[qi * h + a][qj * h + b] = X[a][b]

    m1 = m(0); m4 = m(3); c11 = add(m1, m4)
    m2 = m(1); fin(1, 0, add(m2, m4)); c22 = sub(m1, m2)
    m5 = m(4); c11 = sub(c11, m5)
    m3 = m(2); fin(0, 1, add(m3, m5)); c22 = add(c22, m3)
    m7 = m(6); fin(0, 0, add(c11, m7))
    m6 = m(5); fin(1, 1, add(c22, m6))
    return None if emit is not None else out


class _Sched:
    def __init__(self):
        self.gens = []

    def add(self, gen, units, ticks):
        self.gens.append([gen, units / float(ticks), 0.0])

    def tick(self):
        for e in list(self.gens):
            e[2] += e[1]
            while e[2] >= 1.0:
                e[2] -= 1.0
                try:
                    next(e[0])
                except StopIteration:
                    self.gens.remove(e)
                    break

    def drain(self):
        for e in self.gens:
            for _ in e[0]:
                pass
        self.gens = []


def make(L=2, HQ=64, TN=256, vmem_mb=120, scopes=False, lnrows=16, ln_keep=False, r_phase=2, kv_end=True, wchunks=4,
         lead=0.85, ffn_tile=3, ffn_at='Q', ffn_chain=0, rsq='lax', tail_split=True, wc2_tile=-1, flags=None):
    R = 2 ** L
    P = 7 ** L
    DB = D // R
    TM = R * HQ
    NT = S // TM
    NTN = DB // TN
    CG = 16
    NL1 = 7 if L > 0 else 1
    RA, RW = HQ // 2, DB // 2
    SW = RW // RA
    A_TERMS = _terms(R, True)
    sc = (lambda n: jax.named_scope(n)) if scopes else (lambda n: contextlib.nullcontext())
    CQ, CK, CV = 0, 1, 2

    def kernel(x_hbm, wqkv_hbm, wo_hbm, wr_ref, wg_hbm, wu_hbm, wd_hbm, o_hbm,
               x_v, w_v, wo_v, wg_v, wu_v, wd_v,
               xn_v, pq_v, pk_v, v_v, kv_v, z_v, zg_v, m_v, ost, sem, osem, zsem, wcv, wck, wcq, mc, *xc):
        ns = [0]

        def dma(src, dst):
            c = pltpu.make_async_copy(src, dst, sem.at[ns[0]])
            ns[0] += 1
            return c
        cx = [dma(x_hbm.at[pl.ds(i * TM, TM)], x_v.at[i]) for i in range(NT)]
        wsrc = wqkv_hbm.reshape(R, DB, 3 * D)
        wdst = w_v.reshape(3, R, DB, D)
        rc = DB // wchunks
        cw1 = [dma(wsrc.at[:, pl.ds(j * rc, rc), pl.ds(CV * D, D)], wdst.at[CV, :, pl.ds(j * rc, rc), :]) for j in range(wchunks)]
        cw2 = dma(wqkv_hbm.at[:, pl.ds(CK * D, D)], w_v.at[CK])
        cw3 = dma(wqkv_hbm.at[:, pl.ds(CQ * D, D)], w_v.at[CQ])
        cwo = dma(wo_hbm, wo_v)
        cff = [dma(wg_hbm, wg_v), dma(wu_hbm, wu_v), dma(wd_hbm, wd_v)]
        for c in [cx[0]] + cw1 + cx[1:NT // 2] + [cw2] + cx[NT // 2:] + [cw3, cwo] + cff:
            c.start()

        zS, zL, z2 = (pl.semaphore_read(zsem.at[j]) for j in range(3))

        def operand_sums(load, dst, g0, g1):
            for g in range(g0, g1):
                for t in range(DB // 128):
                    for k in range(NL1):
                        cache = {}

                        def ld(a, b):
                            if (a, b) not in cache:
                                cache[(a, b)] = load(a, b, g, t)
                            return cache[(a, b)]
                        outs = []
                        for eo in range(2):
                            blk = [[_Lazy(lambda a=a, b=b: ld(a, b)[eo]) for b in range(R)] for a in range(R)]
                            lst = []
                            _operands(_level(blk, False, _lazy_add)[k] if L else blk, False, lst)
                            outs.append(lst)
                        n1 = len(outs[0])
                        for j, (e, o) in enumerate(zip(*outs)):
                            r0 = (k * n1 + j) * RW + g * (CG // 2)
                            dst[zS + r0 // RA, pl.ds(r0 % RA, CG // 2), pl.ds(t * 128, 128)] = _pk2(e, o)
                        yield
        n_sums = (DB // CG) * (DB // 128) * NL1
        sch = _Sched()
        TICKS = NTN * P

        def run(gen):
            for _ in gen:
                pass

        def load_w(j):
            def f(a, b, g, t):
                w = pltpu.bitcast(w_v[j, pl.ds(a * DB + g * CG, CG), pl.ds(b * DB + t * 128, 128)], I32)
                return _unp(w, 0), _unp(w, 1)
            return f

        def load_m(a, b, g, t):
            j, r = (b * DB) // 128 + t, a * DB + g * CG
            return m_v[zL + j, pl.ds(r, 8, stride=2), :], m_v[zL + j, pl.ds(r + 1, 8, stride=2), :]

        best = [None, None]
        wr = jnp.broadcast_to(wr_ref[...].astype(F32).reshape(1, D), (8, D))

        def rsqrt(v):
            if rsq == 'lax':
                return lax.rsqrt(v)
            r = pl.reciprocal(jnp.sqrt(v), approx=False)
            return r

        def score(xn, r0):
            n = xn.shape[0]
            rr = jnp.sum(xn.reshape(n // 8, 8, D) * wr[None], axis=-1, keepdims=True)
            for u in range(n // 8):
                ru = rr[u]
                iu = lax.broadcasted_iota(I32, (8, 1), 0) + (r0 + u * 8)
                if best[0] is None:
                    best[0], best[1] = ru, iu
                else:
                    upd = ru > best[0]
                    best[1] = jnp.where(upd, iu, best[1])
                    best[0] = jnp.where(upd, ru, best[0])

        def layernorm(i):
            LR = lnrows
            for g in range(TM // LR):
                r = g * LR
                ld = lambda z: x_v[z + i, pl.ds(r, LR), :].astype(F32)
                mu = jnp.mean(ld(zS), axis=-1, keepdims=True)
                d = ld(zL) - mu
                rstd = rsqrt(jnp.mean(d * d, axis=-1, keepdims=True) + 1e-5)
                xn = (d if ln_keep else ld(z2) - mu) * rstd
                r0 = i * TM + r
                for j in range(D // 128):
                    xn_v[zS + j, pl.ds(r0, LR), :] = xn[:, j * 128:(j + 1) * 128]
                if r_phase == 1:
                    score(xn, r0)
                yield

        def score_tile(i):
            for g in range(TM // 16):
                r0 = i * TM + g * 16
                score(jnp.concatenate([xn_v[zL + j, pl.ds(r0, 16), :] for j in range(D // 128)], axis=1), r0)
                yield

        def comb(terms, get):
            acc = None
            for sg, a, b in terms:
                v = get(a, b)
                acc = (v if sg > 0 else -v) if acc is None else (acc + v if sg > 0 else acc - v)
            return acc

        def lhs_eo(ref, i, p):
            cols = []
            for c in range(DB // 128):
                eo = [comb(A_TERMS[p], lambda a, b: ref[zL + (b * DB) // 128 + c, pl.ds(i * TM + a * HQ + par, HQ // 2, stride=2), :])
                      for par in range(2)]
                cols.append(_pk2(eo[0], eo[1]))
            return jnp.concatenate(cols, axis=1)

        def lhs_nat(ref, i, p):
            v = comb(A_TERMS[p], lambda a, b: jnp.concatenate(
                [ref[zL + (b * DB) // 128 + c, pl.ds(i * TM + a * HQ, HQ), :] for c in range(DB // 128)], axis=1))
            return v.astype(BF16)

        def proj(i, rhs, epi, mode):
            for t in range(NTN):
                def prod(p):
                    if mode == 'first' and t == 0:
                        aw = lhs_eo(xn_v, i, p)
                        xc[i][zS + p] = aw
                        a = _up(aw)
                    elif mode == 'final':
                        a = lhs_nat(pq_v, i, p)
                    else:
                        a = _up(xc[i][zL + p])
                    b = _up(jnp.concatenate([rhs[zL + p * SW + h, :, pl.ds(t * TN, TN)] for h in range(SW)], axis=0))
                    r = _dot(a, b)
                    sch.tick()
                    return r
                _strassen(prod, L, lambda a, b, v: epi(i, a, b * DB + t * TN, v))

        zinit = set()

        def epi_k(i, a, c0, v):
            pk = _phi(v)
            zp = jnp.sum(pk.reshape(HQ // 8, 8, TN), axis=0)
            if c0 not in zinit:
                zinit.add(c0)
                z_v[:, pl.ds(c0, TN)] = zp
            else:
                z_v[:, pl.ds(c0, TN)] += zp
            pk_v[zS + i * R + a, :, pl.ds(c0, TN)] = _pk_blocks(pk)

        def epi_v(i, a, c0, v):
            v_v[zS + i * R + a, :, pl.ds(c0, TN)] = _pk_blocks(v)

        def kv_pass(blocks, first):
            for g in range(D // 128):
                c = pl.ds(g * 128, 128)
                u = lax.dot_general(_up(jnp.concatenate([pk_v[zL + j, :, c] for j in blocks], axis=0)),
                                    _up(jnp.concatenate([v_v[zL + j, :, c] for j in blocks], axis=0)),
                                    (((0,), (0,)), ((), ())), preferred_element_type=F32)
                if first:
                    kv_v[g] = u
                else:
                    kv_v[g] += u

        def epi_q(i, a, c0, v):
            pq = _phi(v)
            for s in range(TN // 128):
                pqs = pq[:, s * 128:(s + 1) * 128]
                den = _dot(pqs.astype(BF16), _up(zg_v[(c0 + s * 128) // 128])) + 1e-6
                pq_v[zS + (c0 + s * 128) // 128, pl.ds(i * TM + a * HQ, HQ), :] = pqs * _rcp(den)

        def epi_o(i, a, c0, v):
            rows = pl.ds(i * TM + a * HQ, HQ)
            xr = jnp.concatenate([xn_v[zL + c0 // 128 + s, rows, :] for s in range(TN // 128)], axis=1)
            ost[rows, pl.ds(c0, TN)] = (v + xr + x_v[i, pl.ds(a * HQ, HQ), pl.ds(c0, TN)].astype(F32)).astype(BF16)

        hmask = (lax.broadcasted_iota(I32, (128, 128), 0) // DH) == (lax.broadcasted_iota(I32, (128, 128), 1) // DH)
        NG = DB // CG

        with sc('p_ln0'):
            cx[0].wait()
            run(layernorm(0))
        with sc('p_wc1'):
            for j in range(wchunks):
                cw1[j].wait()
                run(operand_sums(load_w(CV), wcv, j * NG // wchunks, (j + 1) * NG // wchunks))
        with sc('phV'):
            t2 = wc2_tile % NT
            for i in range(NT):
                if i + 1 < NT:
                    cx[i + 1].wait()
                    sch.add(layernorm(i + 1), TM // lnrows, TICKS * lead)
                if i == t2:
                    cw2.wait()
                    sch.add(operand_sums(load_w(CK), wck, 0, NG), n_sums, TICKS * lead)
                proj(i, wcv, epi_v, 'first')
                sch.drain()

        def zg_pass():
            z = jnp.sum(z_v[...], axis=0, keepdims=True)
            for g in range(D // 128):
                zc = jnp.broadcast_to(z[:, g * 128:(g + 1) * 128], (128, 128)).T
                zg_v[g] = pltpu.bitcast(jnp.where(hmask, zc, 0.0).astype(BF16), I32)

        with sc('phK'):
            cw3.wait()
            sch.add(operand_sums(load_w(CQ), wcq, 0, NG), n_sums, NT * TICKS * lead)
            if r_phase == 2:
                sch.add((None for i in range(NT) for _ in score_tile(i)), S // 16, NT * TICKS * lead)
            for i in range(NT):
                proj(i, wck, epi_k, 'load')
                if not kv_end:
                    kv_pass([i * R + a for a in range(R)], i == 0)
            sch.drain()
            if kv_end:
                kv_pass(list(range(NT * R)), True)
            zg_pass()
            cwo.wait()

        mx = jnp.max(best[0], axis=0, keepdims=True)
        ix = jnp.min(jnp.where(best[0] == mx, best[1], 1 << 30), axis=0, keepdims=True)
        idx = ix[0, 0]
        b16 = pl.multiple_of((idx // 16) * 16, 16)
        sel = lax.broadcasted_iota(I32, (16, D), 0) == idx - b16
        xs = jnp.where(sel, jnp.concatenate([xn_v[zL + j, pl.ds(b16, 16), :] for j in range(D // 128)], axis=1), 0.0).astype(BF16)
        rb = lambda v: v.astype(BF16).astype(F32)
        gate = rb(jax.nn.sigmoid(rb(mx)))

        def ffn_chunk(c, y, FC=512):
            cs = pl.ds(c * FC, FC)
            gg = rb(_dot(xs, wg_v[:, cs]))
            uu = rb(_dot(xs, wu_v[:, cs]))
            h = (rb(gg * jax.nn.sigmoid(gg)) * uu).astype(BF16)
            yy = _dot(h, wd_v[cs, :])
            return yy if y is None else y + yy

        def ffn_finish(y):
            yg = rb(y) * gate
            for j in range(D // 128):
                xn_v[zS + j, pl.ds(b16, 16), :] += yg[:, j * 128:(j + 1) * 128]

        with sc('phQ'):
            y = None
            for i in range(NT):
                if i == 0:
                    for g in range(D // 128):
                        kvm = jnp.where(hmask, kv_v[g], 0.0).astype(BF16)
                        mm = _dot(kvm, wo_v[pl.ds(g * 128, 128), :])
                        for j in range(D // 128):
                            m_v[zS + j, pl.ds(g * 128, 128), :] = mm[:, j * 128:(j + 1) * 128]
                    sch.add(operand_sums(load_m, mc, 0, NG), n_sums, TICKS * lead)
                if ffn_at == 'Q':
                    if i == ffn_tile:
                        for c in cff:
                            c.wait()
                        for c in range(F // 512):
                            y = ffn_chunk(c, y)
                        ffn_finish(y)
                elif ffn_at == 'Qs':
                    if i == 1:
                        for c in cff:
                            c.wait()
                    if 1 <= i <= 7:
                        y = ffn_chunk(i - 1, y)
                        if i == 7:
                            ffn_finish(y)
                proj(i, wcq, epi_q, 'load')
                sch.drain()
        co = []
        with sc('phF'):
            for i in range(NT):
                proj(i, mc, epi_o, 'final')
                parts = 2 if (tail_split and i == NT - 1) else 1
                for h in range(parts):
                    rows = pl.ds(i * TM + h * (TM // parts), TM // parts)
                    c = pltpu.make_async_copy(ost.at[rows], o_hbm.at[rows], osem.at[len(co)])
                    c.start()
                    co.append(c)
        with sc('tail'):
            for c in co:
                c.wait()

    any_spec = pl.BlockSpec(memory_space=pl.ANY)
    V = pltpu.VMEM
    scratch = [
        V((NT, TM, D), BF16), V((3, D, D), BF16), V((D, D), BF16), V((D, F), BF16), V((D, F), BF16), V((F, D), BF16),
        V((D // 128, S, 128), F32), V((D // 128, S, 128), F32), V((NT * R, HQ // 2, D), I32), V((NT * R, HQ // 2, D), I32),
        V((D // 128, 128, 128), F32), V((8, D), F32), V((D // 128, 64, 128), I32), V((D // 128, D, 128), F32),
        V((S, D), BF16),
        pltpu.SemaphoreType.DMA((NT + wchunks + 6,)), pltpu.SemaphoreType.DMA((NT + 1,)), pltpu.SemaphoreType.REGULAR((3,)),
    ] + [V((P * SW, HQ // 2, DB), I32) for _ in range(4)] + [V((P, HQ // 2, DB), I32) for _ in range(NT)]

    def fn(A_x, A_wqkv, A_wo, B_x, B_w_r, B_w_gate, B_w_up, B_w_down):
        del B_x
        out = pl.pallas_call(
            kernel,
            out_shape=jax.ShapeDtypeStruct((S, D), BF16),
            in_specs=[any_spec, any_spec, any_spec, pl.BlockSpec(memory_space=pltpu.VMEM), any_spec, any_spec, any_spec],
            out_specs=any_spec,
            scratch_shapes=scratch,
            compiler_params=pltpu.CompilerParams(vmem_limit_bytes=vmem_mb * 1024 * 1024, flags=flags),
            name="fused",
        )(A_x.reshape(S, D), A_wqkv, A_wo, B_w_r, B_w_gate, B_w_up, B_w_down)
        return out.reshape(1, S, D)
    return fn


_IMPL = make(lead=1.0)


@jax.jit
def pallas_parallel_sum__linear_attn_block__moe_arch_mod__prompt_kernel(
    A_x: jax.Array,
    A_wqkv: jax.Array,
    A_wo: jax.Array,
    B_x: jax.Array,
    B_w_r: jax.Array,
    B_w_gate: jax.Array,
    B_w_up: jax.Array,
    B_w_down: jax.Array,
):
    return _IMPL(A_x, A_wqkv, A_wo, B_x, B_w_r, B_w_gate, B_w_up, B_w_down)
```

```python
import numpy as np
import jax
import jax.numpy as jnp
from jax import lax
from jax.experimental import pallas as pl
from jax.experimental.pallas import tpu as pltpu

S, D, DH, FF = 2048, 1024, 32, 3584
F32, BF16, I32 = jnp.float32, jnp.bfloat16, jnp.int32

LEVELS = 2
R = 2 ** LEVELS
P = 7 ** LEVELS
DB = D // R
HQ = 64
TM = R * HQ
NT = S // TM
RA, RW = HQ // 2, DB // 2
SW = RW // RA
NG = DB // 16
NLT = D // 128
LN_ROWS = 16
W_CHUNKS = 8
MID_WAIT = 28
CQ, CK, CV = 0, 1, 2


def _dot(a, b):
    return jnp.dot(a, b, preferred_element_type=F32)


def _pack(v):
    return pltpu.bitcast(v.astype(BF16), I32)


def _unpack(w):
    return pltpu.bitcast(w, BF16)


def _reciprocal(d):
    r = pl.reciprocal(d, approx=True)
    return r * (2.0 - d * r)


def _phi(t):
    return jnp.where(t > 0, t + 1.0, jnp.exp(t)) + 1e-6


def _round_bf16(v):
    return v.astype(BF16).astype(F32)


def _quad(X, i, j):
    h = len(X) // 2
    return [row[j * h:(j + 1) * h] for row in X[i * h:(i + 1) * h]]


def _level(X, left, add):
    x11, x12, x21, x22 = _quad(X, 0, 0), _quad(X, 0, 1), _quad(X, 1, 0), _quad(X, 1, 1)
    if left:
        return [add(x11, x22, 1), add(x21, x22, 1), x11, x22, add(x11, x12, 1), add(x21, x11, -1), add(x12, x22, -1)]
    return [add(x11, x22, 1), x11, add(x12, x22, -1), add(x21, x11, -1), x22, add(x11, x12, 1), add(x21, x22, 1)]


def _left_terms():
    sym = [[[(1, a, b)] for b in range(R)] for a in range(R)]

    def add(X, Y, sg):
        return [[x + [(sg * s, a, b) for (s, a, b) in y] for x, y in zip(rx, ry)] for rx, ry in zip(X, Y)]

    def rec(X):
        if len(X) == 1:
            return [X[0][0]]
        return [e for o in _level(X, True, add) for e in rec(o)]
    return rec(sym)


LEFT_TERMS = _left_terms()


class _Lazy:
    def __init__(self, f):
        self.f, self.v, self.done = f, None, False

    def get(self):
        if not self.done:
            self.v, self.done = self.f(), True
        return self.v


def _lazy_add(X, Y, s):
    if s > 0:
        return [[_Lazy(lambda x=x, y=y: x.get() + y.get()) for x, y in zip(rx, ry)] for rx, ry in zip(X, Y)]
    return [[_Lazy(lambda x=x, y=y: x.get() - y.get()) for x, y in zip(rx, ry)] for rx, ry in zip(X, Y)]


def _right_operands(blk, out):
    if len(blk) == 1:
        out.append(blk[0][0].get())
        return
    for o in _level(blk, False, _lazy_add):
        _right_operands(o, out)


def _strassen(prod, lvl, emit=None, base=0, i0=0, j0=0):
    if lvl == 0:
        v = prod(base)
        if emit is not None:
            emit(i0, j0, v)
            return None
        return [[v]]
    n = 7 ** (lvl - 1)
    h = 2 ** (lvl - 1)
    m = lambda k: _strassen(prod, lvl - 1, None, base + k * n)
    add = lambda X, Y: [[x + y for x, y in zip(rx, ry)] for rx, ry in zip(X, Y)]
    sub = lambda X, Y: [[x - y for x, y in zip(rx, ry)] for rx, ry in zip(X, Y)]
    out = [[None] * (2 * h) for _ in range(2 * h)]

    def fin(qi, qj, X):
        for a in range(h):
            for b in range(h):
                if emit is not None:
                    emit(i0 + qi * h + a, j0 + qj * h + b, X[a][b])
                else:
                    out[qi * h + a][qj * h + b] = X[a][b]

    m1 = m(0); m4 = m(3); c11 = add(m1, m4)
    m2 = m(1); fin(1, 0, add(m2, m4)); c22 = sub(m1, m2)
    m5 = m(4); c11 = sub(c11, m5)
    m3 = m(2); fin(0, 1, add(m3, m5)); c22 = add(c22, m3)
    m7 = m(6); fin(0, 0, add(c11, m7))
    m6 = m(5); fin(1, 1, add(c22, m6))
    return None if emit is not None else out


class _SideWork:
    def __init__(self):
        self.gens = []
        self.n, self.at = 0, {}

    def add(self, gen, units, ticks):
        self.gens.append([gen, units / float(ticks), 0.0])

    def tick(self):
        self.n += 1
        if self.n in self.at:
            self.at.pop(self.n)()
        for e in list(self.gens):
            e[2] += e[1]
            while e[2] >= 1.0:
                e[2] -= 1.0
                try:
                    next(e[0])
                except StopIteration:
                    self.gens.remove(e)
                    break

    def drain(self):
        for e in self.gens:
            for _ in e[0]:
                pass
        self.gens = []


def _run(gen):
    for _ in gen:
        pass


def _kernel(zero_ref, x_hbm, wqkv_hbm, wo_hbm, wr_ref, wg_hbm, wu_hbm, wd_hbm, o_hbm,
            x_v, w_v, wo_v, wg_v, wu_v, wd_v,
            xn_v, pq_v, pk_v, v_v, kv_v, z_v, zg_v, m_v, ost, fence_v, sem, osem, wcv, wck, wcq, mc, *xc):
    nsem = [0]

    def dma(src, dst):
        c = pltpu.make_async_copy(src, dst, sem.at[nsem[0]])
        nsem[0] += 1
        return c
    cx = [dma(x_hbm.at[pl.ds(i * TM, TM)], x_v.at[i]) for i in range(NT)]
    wsrc = wqkv_hbm.reshape(R, DB, 3 * D)
    wdst = w_v.reshape(3, R, DB, D)
    rc = DB // W_CHUNKS
    cwv = [dma(wsrc.at[:, pl.ds(j * rc, rc), pl.ds(CV * D, D)], wdst.at[CV, :, pl.ds(j * rc, rc), :])
           for j in range(W_CHUNKS)]
    cwk = dma(wqkv_hbm.at[:, pl.ds(CK * D, D)], w_v.at[CK])
    cwq = dma(wqkv_hbm.at[:, pl.ds(CQ * D, D)], w_v.at[CQ])
    cwo = dma(wo_hbm, wo_v)
    cff = [dma(wg_hbm, wg_v), dma(wu_hbm, wu_v), dma(wd_hbm, wd_v)]
    cfence = dma(x_hbm.at[pl.ds(0, 16)], fence_v)
    for c in [cx[0]] + cwv + cx[1:NT // 2] + [cwk] + cx[NT // 2:] + [cwq, cwo] + cff + [cfence]:
        c.start()

    zS, zL, z2 = (zero_ref[j] for j in range(3))
    side = _SideWork()

    def operand_sums(load, dst, g0, g1):
        for g in range(g0, g1):
            for t in range(DB // 128):
                for k in range(7):
                    cache = {}

                    def ld(a, b):
                        if (a, b) not in cache:
                            cache[(a, b)] = load(a, b, g, t)
                        return cache[(a, b)]
                    blk = [[_Lazy(lambda a=a, b=b: ld(a, b)) for b in range(R)] for a in range(R)]
                    ops = []
                    _right_operands(_level(blk, False, _lazy_add)[k], ops)
                    for j, v in enumerate(ops):
                        r0 = (k * len(ops) + j) * RW + g * 8
                        dst[zS + r0 // RA, pl.ds(r0 % RA, 8), pl.ds(t * 128, 128)] = _pack(v)
                    yield
    n_sums = NG * (DB // 128) * 7

    def load_w(j):
        return lambda a, b, g, t: w_v[j, pl.ds(a * DB + g * 16, 16), pl.ds(b * DB + t * 128, 128)].astype(F32)

    def load_m(a, b, g, t):
        return m_v[zL + (b * DB) // 128 + t, pl.ds(a * DB + g * 16, 16), :]

    best = [None, None]
    wr = jnp.broadcast_to(wr_ref[...].astype(F32).reshape(1, D), (8, D))

    def layernorm(i):
        for g in range(TM // LN_ROWS):
            r = g * LN_ROWS
            ld = lambda z: x_v[z + i, pl.ds(r, LN_ROWS), :].astype(F32)
            mu = jnp.mean(ld(zS), axis=-1, keepdims=True)
            d = ld(zL) - mu
            rstd = lax.rsqrt(jnp.mean(d * d, axis=-1, keepdims=True) + 1e-5)
            xn = (ld(z2) - mu) * rstd
            for j in range(NLT):
                xn_v[zS + j, pl.ds(i * TM + r, LN_ROWS), :] = xn[:, j * 128:(j + 1) * 128]
            yield

    def router_scores():
        for r0 in range(0, S, 16):
            xn = jnp.concatenate([xn_v[zL + j, pl.ds(r0, 16), :] for j in range(NLT)], axis=1)
            rr = jnp.sum(xn.reshape(2, 8, D) * wr[None], axis=-1, keepdims=True)
            for u in range(2):
                ru = rr[u]
                iu = lax.broadcasted_iota(I32, (8, 1), 0) + (r0 + u * 8)
                if best[0] is None:
                    best[0], best[1] = ru, iu
                else:
                    upd = ru > best[0]
                    best[1] = jnp.where(upd, iu, best[1])
                    best[0] = jnp.where(upd, ru, best[0])
            yield

    def left_operand(ref, i, p):
        acc = None
        for sg, a, b in LEFT_TERMS[p]:
            v = jnp.concatenate([ref[zL + (b * DB) // 128 + c, pl.ds(i * TM + a * HQ, HQ), :]
                                 for c in range(DB // 128)], axis=1)
            acc = (v if sg > 0 else -v) if acc is None else (acc + v if sg > 0 else acc - v)
        return acc

    def proj(i, rhs, epilogue, mode):
        def prod(p):
            if mode == 'first':
                aw = _pack(left_operand(xn_v, i, p))
                xc[i][zS + p] = aw
                a = _unpack(aw)
            elif mode == 'final':
                a = left_operand(pq_v, i, p).astype(BF16)
            else:
                a = _unpack(xc[i][zL + p])
            b = _unpack(jnp.concatenate([rhs[zL + p * SW + h, :, pl.ds(0, DB)] for h in range(SW)], axis=0))
            r = _dot(a, b)
            side.tick()
            return r
        _strassen(prod, LEVELS, lambda a, b, v: epilogue(i, a, b * DB, v))

    z_started = set()

    def epi_v(i, a, c0, v):
        v_v[zS + i * R + a, :, pl.ds(c0, DB)] = _pack(v)

    def epi_k(i, a, c0, v):
        pk = _phi(v)
        zp = jnp.sum(pk.reshape(HQ // 8, 8, DB), axis=0)
        if c0 not in z_started:
            z_started.add(c0)
            z_v[:, pl.ds(c0, DB)] = zp
        else:
            z_v[:, pl.ds(c0, DB)] += zp
        pk_v[zS + i * R + a, :, pl.ds(c0, DB)] = _pack(pk)

    def epi_q(i, a, c0, v):
        pq = _phi(v)
        for s in range(DB // 128):
            pqs = pq[:, s * 128:(s + 1) * 128]
            den = _dot(pqs.astype(BF16), _unpack(zg_v[c0 // 128 + s])) + 1e-6
            pq_v[zS + c0 // 128 + s, pl.ds(i * TM + a * HQ, HQ), :] = pqs * _reciprocal(den)

    def epi_out(i, a, c0, v):
        rows = pl.ds(i * TM + a * HQ, HQ)
        xn = jnp.concatenate([xn_v[zL + c0 // 128 + s, rows, :] for s in range(DB // 128)], axis=1)
        ost[rows, pl.ds(c0, DB)] = (v + xn + x_v[i, pl.ds(a * HQ, HQ), pl.ds(c0, DB)].astype(F32)).astype(BF16)

    same_head = (lax.broadcasted_iota(I32, (128, 128), 0) // DH) == (lax.broadcasted_iota(I32, (128, 128), 1) // DH)

    cx[0].wait()
    _run(layernorm(0))
    for j in range(W_CHUNKS):
        cwv[j].wait()
        _run(operand_sums(load_w(CV), wcv, j * NG // W_CHUNKS, (j + 1) * NG // W_CHUNKS))

    for i in range(NT):
        if i == 0:
            def second_tile():
                cx[1].wait()
                side.add(layernorm(1), TM // LN_ROWS, P - MID_WAIT)
            side.at[side.n + MID_WAIT] = second_tile
        elif i + 1 < NT:
            cx[i + 1].wait()
            side.add(layernorm(i + 1), TM // LN_ROWS, P)
        if i == NT - 1:
            cwk.wait()
            side.add(operand_sums(load_w(CK), wck, 0, NG), n_sums, P)
        proj(i, wcv, epi_v, 'first')
        side.drain()

    cwq.wait()
    side.add(operand_sums(load_w(CQ), wcq, 0, NG), n_sums, NT * P)
    side.add(router_scores(), S // 16, NT * P)
    for i in range(NT):
        proj(i, wck, epi_k, 'load')
    side.drain()
    for g in range(NLT):
        c = pl.ds(g * 128, 128)
        kv_v[g] = lax.dot_general(_unpack(jnp.concatenate([pk_v[zL + j, :, c] for j in range(NT * R)], axis=0)),
                                  _unpack(jnp.concatenate([v_v[zL + j, :, c] for j in range(NT * R)], axis=0)),
                                  (((0,), (0,)), ((), ())), preferred_element_type=F32)
    z = jnp.sum(z_v[...], axis=0, keepdims=True)
    for g in range(NLT):
        zc = jnp.broadcast_to(z[:, g * 128:(g + 1) * 128], (128, 128)).T
        zg_v[g] = _pack(jnp.where(same_head, zc, 0.0))
    cwo.wait()

    mx = jnp.max(best[0], axis=0, keepdims=True)
    idx = jnp.min(jnp.where(best[0] == mx, best[1], 1 << 30), axis=0, keepdims=True)[0, 0]
    idx = jnp.clip(idx, 0, S - 1)
    b16 = pl.multiple_of((idx // 16) * 16, 16)
    sel = lax.broadcasted_iota(I32, (16, D), 0) == idx - b16
    xs = jnp.where(sel, jnp.concatenate([xn_v[zL + j, pl.ds(b16, 16), :] for j in range(NLT)], axis=1), 0.0)
    xs = xs.astype(BF16)
    gate = _round_bf16(jax.nn.sigmoid(_round_bf16(mx)))

    def routed_ffn():
        y = None
        for j in range(FF // 128):
            cs = pl.ds(j * 128, 128)
            g_ = _round_bf16(_dot(xs, wg_v[:, cs]))
            yield
            u_ = _round_bf16(_dot(xs, wu_v[:, cs]))
            yield
            h = (_round_bf16(g_ * jax.nn.sigmoid(g_)) * u_).astype(BF16)
            yy = _dot(h, wd_v[cs, :])
            y = yy if y is None else y + yy
            yield
        yg = _round_bf16(y) * gate
        for j in range(NLT):
            xn_v[zS + j, pl.ds(b16, 16), :] += yg[:, j * 128:(j + 1) * 128]
        yield

    ffn = routed_ffn()
    ffn_left = 3 * (FF // 128) + 1
    for i in range(NT):
        if i == 0:
            for g in range(NLT):
                kvm = jnp.where(same_head, kv_v[g], 0.0).astype(BF16)
                mm = _dot(kvm, wo_v[pl.ds(g * 128, 128), :])
                for j in range(NLT):
                    m_v[zS + j, pl.ds(g * 128, 128), :] = mm[:, j * 128:(j + 1) * 128]
            side.add(operand_sums(load_m, mc, 0, NG), n_sums, P)
        else:
            if i == 1:
                for c in cff:
                    c.wait()
            n = -(-ffn_left // (NT - i))
            ffn_left -= n
            side.add((next(ffn) for _ in range(n)), n, P * 0.95)
        proj(i, wcq, epi_q, 'load')
        side.drain()

    cfence.wait()
    outs = []
    for i in range(NT):
        proj(i, mc, epi_out, 'final')
        parts = 2 if i == NT - 1 else 1
        for h in range(parts):
            rows = pl.ds(i * TM + h * (TM // parts), TM // parts)
            c = pltpu.make_async_copy(ost.at[rows], o_hbm.at[rows], osem.at[len(outs)])
            c.start()
            outs.append(c)
    for c in outs:
        c.wait()


@jax.jit
def pallas_parallel_sum__linear_attn_block__moe_arch_mod__prompt_kernel(
    A_x: jax.Array,
    A_wqkv: jax.Array,
    A_wo: jax.Array,
    B_x: jax.Array,
    B_w_r: jax.Array,
    B_w_gate: jax.Array,
    B_w_up: jax.Array,
    B_w_down: jax.Array,
):
    del B_x
    V = pltpu.VMEM
    hbm = pl.BlockSpec(memory_space=pl.ANY)
    scratch = [
        V((NT, TM, D), BF16), V((3, D, D), BF16), V((D, D), BF16),
        V((D, FF), BF16), V((D, FF), BF16), V((FF, D), BF16),
        V((NLT, S, 128), F32), V((NLT, S, 128), F32),
        V((NT * R, RA, D), I32), V((NT * R, RA, D), I32),
        V((NLT, 128, 128), F32), V((8, D), F32), V((NLT, 64, 128), I32), V((NLT, D, 128), F32),
        V((S, D), BF16), V((16, D), BF16),
        pltpu.SemaphoreType.DMA((NT + W_CHUNKS + 7,)), pltpu.SemaphoreType.DMA((NT + 1,)),
    ] + [V((P * SW, RA, DB), I32) for _ in range(4)] + [V((P, RA, DB), I32) for _ in range(NT)]
    out = pl.pallas_call(
        _kernel,
        out_shape=jax.ShapeDtypeStruct((S, D), BF16),
        in_specs=[pl.BlockSpec(memory_space=pltpu.SMEM), hbm, hbm, hbm, pl.BlockSpec(memory_space=pltpu.VMEM),
                  hbm, hbm, hbm],
        out_specs=hbm,
        scratch_shapes=scratch,
        compiler_params=pltpu.CompilerParams(vmem_limit_bytes=120 * 1024 * 1024),
        name="fused_linear_attn_mod",
    )(np.array([0, 0, 0, 1], np.int32), A_x.reshape(S, D), A_wqkv, A_wo, B_w_r, B_w_gate, B_w_up, B_w_down)
    return out.reshape(1, S, D)
```
